```python
import jax
import jax.numpy as jnp

def _softmax(x, axis=-1):
    return jax.nn.softmax(x, axis=axis)
def _gelu(x):
    return jax.nn.gelu(x, approximate=True)
def _silu(x):
    return jax.nn.silu(x)
def _sigmoid(x):
    return jax.nn.sigmoid(x)
def _layernorm(x, axis=-1, eps=1e-5):
    m = jnp.mean(x, axis=axis, keepdims=True)
    v = jnp.var(x, axis=axis, keepdims=True)
    return (x - m) / jnp.sqrt(v + eps)
def _scatter_add(tgt, idx, src, axis=0):
    return tgt.at[idx].add(src)
def _segment_sum(src, seg, n):
    return jax.ops.segment_sum(src, seg, n)
class _Rng:
    def __init__(self, key):
        self._k = key
    def _next(self):
        self._k, sub = jax.random.split(self._k)
        return sub
    def normal(self, shape):
        return jax.random.normal(self._next(), shape, dtype=jnp.bfloat16)
    def randint(self, lo, hi, shape):
        return jax.random.randint(self._next(), shape, lo, hi, dtype=jnp.int32)
    def uniform(self, shape, lo=0.0, hi=1.0):
        return jax.random.uniform(self._next(), shape, jnp.bfloat16, lo, hi)
    def permutation(self, n):
        return jax.random.permutation(self._next(), n)


kernel_name = 'gated_mix__sliding_block_cached__dense_activation_gelu__decode'

def setup_inputs():
    _rng = _Rng(jax.random.key(int.from_bytes(__import__("os").urandom(4), "little")))
    _w = (lambda a: (lambda t: t.astype(jnp.bfloat16) if jnp.issubdtype(t.dtype, jnp.floating) else t)(jnp.asarray(a)))
    def _A_setup():
        B, Sq, D = 1, 1, 640
        Hq, Hkv, Sk, Dh = 32, 32, 32768, 192
        assert Hq % Hkv == 0, (Hq, Hkv)
        return {
            "x": _w((lambda *s: _rng.normal(s) * 0.05)(B, Sq, D)),
            "k_cache": _w((lambda *s: _rng.normal(s) * 0.05)(B, Hkv, Sk, Dh)),
            "v_cache": _w((lambda *s: _rng.normal(s) * 0.05)(B, Hkv, Sk, Dh)),
            "wq": _w((lambda *s: _rng.normal(s) * 0.05)(D, Hq * Dh) * (D ** -0.5)),
            "wo": _w((lambda *s: _rng.normal(s) * 0.05)(Hq * Dh, D) * ((Hq * Dh) ** -0.5)),
        }
    _A_in = _A_setup()

    def _B_setup():
        B, S, D, F = 1, 1, 640, 1536
        return {
            "x": _w((lambda *s: _rng.normal(s) * 0.05)(B, S, D)),
            "w1": _w((lambda *s: _rng.normal(s) * 0.05)(D, F) * (D ** -0.5)),
            "b1": _w((lambda *s: _rng.normal(s) * 0.05)(F) * 0.01),
            "w2": _w((lambda *s: _rng.normal(s) * 0.05)(F, D) * (F ** -0.5)),
            "b2": _w((lambda *s: _rng.normal(s) * 0.05)(D) * 0.01),
        }
    _B_in = _B_setup()

    return {
        "A_x": _A_in["x"],
        "A_k_cache": _A_in["k_cache"],
        "A_v_cache": _A_in["v_cache"],
        "A_wq": _A_in["wq"],
        "A_wo": _A_in["wo"],
        "B_x": _B_in["x"],
        "B_w1": _B_in["w1"],
        "B_b1": _B_in["b1"],
        "B_w2": _B_in["w2"],
        "B_b2": _B_in["b2"],
        "gate_w": _w((lambda *s: _rng.normal(s) * 0.05)(640)),
    }

def reference(A_x, A_k_cache, A_v_cache, A_wq, A_wo, B_x, B_w1, B_b1, B_w2, B_b2, gate_w):
    def _A_ref(x, k_cache, v_cache, wq, wo):
        B, Sq, D = x.shape
        Hq, Dh = 32, 192
        Hkv, Sk = k_cache.shape[1], k_cache.shape[2]
        W = min(4096, max(256, Sk // 4))
        rep = Hq // Hkv
        q = (lambda x, *d: x.transpose(*d))((x @ wq).reshape(B, Sq, Hq, Dh), 0, 2, 1, 3)
        k = jnp.repeat(k_cache[:, :, Sk - W:, :], rep, axis=1)
        v = jnp.repeat(v_cache[:, :, Sk - W:, :], rep, axis=1)
        scores = jnp.einsum("bhqd,bhkd->bhqk", q, k) * (Dh ** -0.5)
        p = _softmax(scores, axis=-1)
        o = jnp.einsum("bhqk,bhkd->bhqd", p, v)
        return (lambda x, *d: x.transpose(*d))(o, 0, 2, 1, 3).reshape(B, Sq, Hq * Dh) @ wo

    def _B_ref(x, w1, b1, w2, b2):
        h = jnp.einsum("bsd,df->bsf", x, w1) + b1
        h = _gelu(h)
        return jnp.einsum("bsf,fd->bsd", h, w2) + b2

    x = A_x
    g = _sigmoid((x * gate_w).sum(-1, keepdims=True))
    a = _A_ref(x, A_k_cache, A_v_cache, A_wq, A_wo)
    b = _B_ref(x, B_w1, B_b1, B_w2, B_b2)
    return g * a + (1 - g) * b
```

```python
import functools

import jax
import jax.numpy as jnp
from jax.experimental import pallas as pl
from jax.experimental.pallas import tpu as pltpu

_HQ, _DH = 32, 192
_M = 8


def _pieces(nr, nc, R, C, order):
    if order == "row":
        return [(r, c) for r in range(nr // R) for c in range(nc // C)]
    return [(r, c) for c in range(nc // C) for r in range(nr // R)]


def make(NP=2, R=32, C=512, order="row", M=_M, RQ=32, RO=32, R1=16, R2=32, NW2=6, vmem_mb=100):
    def fn(A_x, A_k_cache, A_v_cache, A_wq, A_wo, B_x, B_w1, B_b1, B_w2, B_b2, gate_w):
        del B_x
        _, _, D = A_x.shape
        _, Hkv, Sk, Dh = A_k_cache.shape
        assert Hkv == _HQ and Dh == _DH
        F = B_w1.shape[1]
        W = min(4096, max(256, Sk // 4))
        PW = 2 * Dh
        NPAIR = _HQ // 2
        scale = Dh ** -0.5
        f32, bf16 = jnp.float32, jnp.bfloat16
        W2R = F // NW2

        def kernel(x_hbm, kt_hbm, vt_hbm, wq_hbm, wo_hbm, w1_hbm, b1_hbm, w2_hbm, b2_hbm, g_hbm,
                   o_ref,
                   xs, gs, b1s, b2s, w1s, w2s, wqb, kb, vb, wob,
                   sem_small, sem_w1, sem_w2, sem_wq, sem_k, sem_v, sem_wo):

            def start_qk(j, slot):
                col0 = pl.multiple_of(j * PW, 128)
                for i in range(D // RQ):
                    pltpu.make_async_copy(
                        wq_hbm.at[pl.ds(i * RQ, RQ), pl.ds(col0, PW)],
                        wqb.at[slot, pl.ds(i * RQ, RQ), :], sem_wq.at[slot]).start(priority=i % 2)
                for i, (r, c) in enumerate(_pieces(PW, W, R, C, order)):
                    row0 = pl.multiple_of(j * PW + r * R, 8)
                    pltpu.make_async_copy(
                        kt_hbm.at[pl.ds(row0, R), pl.ds(Sk - W + c * C, C)],
                        kb.at[slot, pl.ds(r * R, R), pl.ds(c * C, C)], sem_k.at[slot]).start(priority=i % 2)

            def start_v(j, slot):
                for i, (r, c) in enumerate(_pieces(PW, W, R, C, order)):
                    row0 = pl.multiple_of(j * PW + r * R, 8)
                    pltpu.make_async_copy(
                        vt_hbm.at[pl.ds(row0, R), pl.ds(Sk - W + c * C, C)],
                        vb.at[slot, pl.ds(r * R, R), pl.ds(c * C, C)], sem_v.at[slot]).start(priority=i % 2)
                for i in range(PW // RO):
                    row0 = pl.multiple_of(j * PW + i * RO, 8)
                    pltpu.make_async_copy(
                        wo_hbm.at[pl.ds(row0, RO), :],
                        wob.at[slot, pl.ds(i * RO, RO), :], sem_wo.at[slot]).start(priority=i % 2)

            def start_w2():
                for i in range(F // R2):
                    pltpu.make_async_copy(
                        w2_hbm.at[pl.ds(i * R2, R2), :], w2s.at[pl.ds(i * R2, R2), :],
                        sem_w2.at[(i * R2) // W2R]).start(priority=i % 2)

            def wait_all(buf, sem):
                pltpu.make_async_copy(buf, buf, sem).wait()

            small = [pltpu.make_async_copy(x_hbm, xs, sem_small.at[0]),
                     pltpu.make_async_copy(g_hbm, gs, sem_small.at[1]),
                     pltpu.make_async_copy(b1_hbm, b1s, sem_small.at[2]),
                     pltpu.make_async_copy(b2_hbm, b2s, sem_small.at[3])]
            for cp in small:
                cp.start()
            for i in range(D // R1):
                pltpu.make_async_copy(w1_hbm.at[pl.ds(i * R1, R1), :], w1s.at[pl.ds(i * R1, R1), :],
                                      sem_w1.at[0]).start(priority=i % 2)
            for j in range(NP):
                start_qk(j, j)
                start_v(j, j)

            for cp in small:
                cp.wait()
            xv = xs[0].astype(f32)
            g = jax.nn.sigmoid(jnp.sum(xv * gs[...].astype(f32).reshape(1, D), axis=-1, keepdims=True))
            x8 = jnp.broadcast_to(xv, (M, D)).astype(bf16)

            wait_all(w1s, sem_w1.at[0])
            h = jnp.dot(x8, w1s[...], preferred_element_type=f32) + b1s[...].astype(f32).reshape(1, F)
            h = jax.nn.gelu(h, approximate=True).astype(bf16)

            row = jax.lax.broadcasted_iota(jnp.int32, (M, PW), 0)
            col = jax.lax.broadcasted_iota(jnp.int32, (M, PW), 1)
            diag = ((row == 0) & (col < Dh)) | ((row == 1) & (col >= Dh))

            def body(j, acc):
                slot = j % NP
                wait_all(wqb.at[slot], sem_wq.at[slot])
                wait_all(kb.at[slot], sem_k.at[slot])
                q = jnp.dot(x8, wqb[slot], preferred_element_type=f32)
                qd = jnp.where(diag, q, 0.0).astype(bf16)
                s = jnp.dot(qd, kb[slot], preferred_element_type=f32) * scale
                m = jnp.max(s, axis=-1, keepdims=True)
                p = jnp.exp(s - m)
                l = jnp.sum(p, axis=-1, keepdims=True)
                pb = p.astype(bf16)

                @pl.when(j + NP < NPAIR)
                def _():
                    start_qk(j + NP, slot)

                @pl.when(j + NP == NPAIR)
                def _():
                    start_w2()

                wait_all(vb.at[slot], sem_v.at[slot])
                wait_all(wob.at[slot], sem_wo.at[slot])
                o = jax.lax.dot_general(pb, vb[slot], (((1,), (1,)), ((), ())),
                                        preferred_element_type=f32)
                o = jnp.where(diag, o / l, 0.0).astype(bf16)
                acc = acc + jnp.dot(o, wob[slot], preferred_element_type=f32)

                @pl.when(j + NP < NPAIR)
                def _():
                    start_v(j + NP, slot)
                return acc

            acc = jax.lax.fori_loop(0, NPAIR, body, jnp.zeros((M, D), f32))
            a = jnp.sum(acc, axis=0, keepdims=True)

            b = jnp.zeros((M, D), f32)
            for c in range(NW2):
                wait_all(w2s.at[pl.ds(c * W2R, W2R), :], sem_w2.at[c])
                b = b + jnp.dot(h[:, c * W2R:(c + 1) * W2R], w2s[c * W2R:(c + 1) * W2R, :],
                                preferred_element_type=f32)
            b = b[0:1] + b2s[...].astype(f32).reshape(1, D)
            o_ref[0] = (g * a + (1.0 - g) * b).astype(o_ref.dtype)

        kt = jnp.transpose(A_k_cache, (0, 1, 3, 2)).reshape(Hkv * Dh, Sk)
        vt = jnp.transpose(A_v_cache, (0, 1, 3, 2)).reshape(Hkv * Dh, Sk)
        hbm = pl.BlockSpec(memory_space=pl.ANY)
        DMA = pltpu.SemaphoreType.DMA
        return pl.pallas_call(
            kernel,
            out_shape=jax.ShapeDtypeStruct((1, 1, D), A_x.dtype),
            in_specs=[hbm] * 10,
            out_specs=pl.BlockSpec(memory_space=pltpu.VMEM),
            scratch_shapes=[
                pltpu.VMEM((1, 1, D), bf16), pltpu.VMEM((D,), bf16),
                pltpu.VMEM((F,), bf16), pltpu.VMEM((D,), bf16),
                pltpu.VMEM((D, F), bf16), pltpu.VMEM((F, D), bf16),
                pltpu.VMEM((NP, D, PW), bf16),
                pltpu.VMEM((NP, PW, W), bf16), pltpu.VMEM((NP, PW, W), bf16),
                pltpu.VMEM((NP, PW, D), bf16),
                DMA((4,)), DMA((1,)), DMA((NW2,)), DMA((NP,)), DMA((NP,)), DMA((NP,)), DMA((NP,)),
            ],
            compiler_params=pltpu.CompilerParams(vmem_limit_bytes=vmem_mb << 20),
        )(A_x, kt, vt, A_wq, A_wo, B_w1, B_b1, B_w2, B_b2, gate_w)
    return fn


@jax.jit
def pallas_gated_mix__sliding_block_cached__dense_activation_gelu__decode_kernel(
    A_x, A_k_cache, A_v_cache, A_wq, A_wo, B_x, B_w1, B_b1, B_w2, B_b2, gate_w
):
    return make()(A_x, A_k_cache, A_v_cache, A_wq, A_wo, B_x, B_w1, B_b1, B_w2, B_b2, gate_w)
```

```python
import functools

import jax
import jax.numpy as jnp
from jax import lax
from jax.experimental import pallas as pl
from jax.experimental.pallas import tpu as pltpu

_HQ, _DH = 32, 192
_M = 8


class _Null:
    def __enter__(self): return None
    def __exit__(self, *a): return False


def make(NP=2, R=32, C=512, M=_M, RQ=32, RO=32, R1=16, R2=32, NW2=6, vmem_mb=100,
         compute=True, scopes=False, nobounds=False, wsplit="half", U=1):
    def fn(A_x, A_k_cache, A_v_cache, A_wq, A_wo, B_x, B_w1, B_b1, B_w2, B_b2, gate_w):
        del B_x
        _, _, D = A_x.shape
        _, Hkv, Sk, Dh = A_k_cache.shape
        assert Hkv == _HQ and Dh == _DH
        F = B_w1.shape[1]
        W = min(4096, max(256, Sk // 4))
        PW = 2 * Dh
        NPAIR = _HQ // 2
        scale = Dh ** -0.5
        f32, bf16 = jnp.float32, jnp.bfloat16
        W2R = F // NW2
        NC = W // C
        NR = PW // R
        NKV = NR * NC
        NQ, NO = D // RQ, PW // RO
        scope = (lambda n: jax.named_scope(n)) if scopes else (lambda n: _Null())

        def kernel(x_hbm, kt_hbm, vt_hbm, wq_hbm, wo_hbm, w1_hbm, b1_hbm, w2_hbm, b2_hbm, g_hbm,
                   o_ref,
                   xs, gs, b1s, b2s, w1s, w2s, wqb, kb, vb, wob,
                   sem_small, sem_w1, sem_w2, sem_wq, sem_k, sem_v, sem_wo):

            def loop(n, f):
                if n <= 0:
                    return
                lax.fori_loop(0, n, lambda i, c: (f(i), c)[1], 0, unroll=U)

            def start_pair(j, slot):
                col0 = pl.multiple_of(j * PW, 128)

                def wq_piece(i):
                    r0 = pl.multiple_of(i * RQ, 8)
                    pltpu.make_async_copy(
                        wq_hbm.at[pl.ds(r0, RQ), pl.ds(col0, PW)],
                        wqb.at[slot, pl.ds(r0, RQ), :], sem_wq.at[slot]).start(priority=0)

                def wo_piece(i):
                    r0 = pl.multiple_of(j * PW + i * RO, 8)
                    pltpu.make_async_copy(
                        wo_hbm.at[pl.ds(r0, RO), :],
                        wob.at[slot, pl.ds(pl.multiple_of(i * RO, 8), RO), :],
                        sem_wo.at[slot]).start(priority=1)

                nmin = min(NQ, NO)
                loop(nmin, lambda i: (wq_piece(i), wo_piece(i)))
                if NQ > nmin:
                    loop(NQ - nmin, lambda i: wq_piece(i + nmin))
                if NO > nmin:
                    loop(NO - nmin, lambda i: wo_piece(i + nmin))

                def kv_piece(i):
                    r, c = i // NC, i % NC
                    r0 = pl.multiple_of(r * R, 8)
                    c0 = pl.multiple_of(c * C, 128)
                    row0 = pl.multiple_of(j * PW + r * R, 8)
                    src = (pl.ds(row0, R), pl.ds(pl.multiple_of(Sk - W + c * C, 128), C))
                    dst = (slot, pl.ds(r0, R), pl.ds(c0, C))
                    pltpu.make_async_copy(kt_hbm.at[src], kb.at[dst], sem_k.at[slot]).start(priority=0)
                    pltpu.make_async_copy(vt_hbm.at[src], vb.at[dst], sem_v.at[slot]).start(priority=1)

                loop(NKV, kv_piece)

            def start_split(hbm, buf, rows, sem_of_row):
                n = hbm.shape[0] // rows
                assert n % 2 == 0
                if wsplit == "half":
                    def piece(i):
                        for t in range(2):
                            r0 = pl.multiple_of((i + t * (n // 2)) * rows, 8)
                            pltpu.make_async_copy(hbm.at[pl.ds(r0, rows), :], buf.at[pl.ds(r0, rows), :],
                                                  sem_of_row(r0)).start(priority=t)
                else:
                    def piece(i):
                        for t in range(2):
                            r0 = pl.multiple_of((2 * i + t) * rows, 8)
                            pltpu.make_async_copy(hbm.at[pl.ds(r0, rows), :], buf.at[pl.ds(r0, rows), :],
                                                  sem_of_row(r0)).start(priority=t)
                loop(n // 2, piece)

            def wait_all(buf, sem):
                pltpu.make_async_copy(buf, buf, sem).wait()

            small = [pltpu.make_async_copy(x_hbm, xs, sem_small.at[0]),
                     pltpu.make_async_copy(g_hbm, gs, sem_small.at[1]),
                     pltpu.make_async_copy(b1_hbm, b1s, sem_small.at[2]),
                     pltpu.make_async_copy(b2_hbm, b2s, sem_small.at[3])]
            with scope("pro_issue"):
                for i, cp in enumerate(small):
                    cp.start(priority=i % 2)
                start_split(w1_hbm, w1s, R1, lambda r0: sem_w1.at[0])
                start_pair(0, 0)

            with scope("pro_compute"):
                for cp in small:
                    cp.wait()
                xv = xs[0].astype(f32)
                g = jax.nn.sigmoid(jnp.sum(xv * gs[...].astype(f32).reshape(1, D), axis=-1, keepdims=True))
                x8 = jnp.broadcast_to(xv, (M, D)).astype(bf16)

                wait_all(w1s, sem_w1.at[0])
                if compute:
                    h = jnp.dot(x8, w1s[...], preferred_element_type=f32) + b1s[...].astype(f32).reshape(1, F)
                    h = jax.nn.gelu(h, approximate=True).astype(bf16)
                else:
                    h = jnp.zeros((M, F), bf16)

            with scope("pro_issue2"):
                for j in range(1, NP):
                    start_pair(j, j)

            row = jax.lax.broadcasted_iota(jnp.int32, (M, PW), 0)
            col = jax.lax.broadcasted_iota(jnp.int32, (M, PW), 1)
            diag = ((row == 0) & (col < Dh)) | ((row == 1) & (col >= Dh))

            def body(j, acc):
                slot = j % NP
                with scope("waitK"):
                    wait_all(wqb.at[slot], sem_wq.at[slot])
                    wait_all(kb.at[slot], sem_k.at[slot])
                if compute:
                    with scope("QK"):
                        q = jnp.dot(x8, wqb[slot], preferred_element_type=f32)
                        qd = jnp.where(diag, q, 0.0).astype(bf16)
                        s = jnp.dot(qd, kb[slot], preferred_element_type=f32) * scale
                        m = jnp.max(s, axis=-1, keepdims=True)
                        p = jnp.exp(s - m)
                        l = jnp.sum(p, axis=-1, keepdims=True)
                        pb = p.astype(bf16)
                with scope("waitV"):
                    wait_all(vb.at[slot], sem_v.at[slot])
                    wait_all(wob.at[slot], sem_wo.at[slot])
                if compute:
                    with scope("PV"):
                        o = jax.lax.dot_general(pb, vb[slot], (((1,), (1,)), ((), ())),
                                                preferred_element_type=f32)
                        o = jnp.where(diag, o / l, 0.0).astype(bf16)
                        acc = acc + jnp.dot(o, wob[slot], preferred_element_type=f32)

                with scope("issue"):
                    @pl.when(j + NP < NPAIR)
                    def _():
                        start_pair(j + NP, slot)

                    @pl.when(j + NP == NPAIR + 1)
                    def _():
                        start_split(w2_hbm, w2s, R2, lambda r0: sem_w2.at[r0 // W2R])
                return acc

            acc = jax.lax.fori_loop(0, NPAIR, body, jnp.zeros((M, D), f32))
            a = jnp.sum(acc, axis=0, keepdims=True)

            b = jnp.zeros((M, D), f32)
            order = list(range(NW2))
            if wsplit == "half":
                order = [c + t * (NW2 // 2) for c in range(NW2 // 2) for t in range(2)]
            for c in order:
                with scope("waitW2"):
                    wait_all(w2s.at[pl.ds(c * W2R, W2R), :], sem_w2.at[c])
                if compute:
                    b = b + jnp.dot(h[:, c * W2R:(c + 1) * W2R], w2s[c * W2R:(c + 1) * W2R, :],
                                    preferred_element_type=f32)
            b = b[0:1] + b2s[...].astype(f32).reshape(1, D)
            o_ref[0] = (g * a + (1.0 - g) * b).astype(o_ref.dtype)

        kt = jnp.transpose(A_k_cache, (0, 1, 3, 2)).reshape(Hkv * Dh, Sk)
        vt = jnp.transpose(A_v_cache, (0, 1, 3, 2)).reshape(Hkv * Dh, Sk)
        hbm = pl.BlockSpec(memory_space=pl.ANY)
        DMA = pltpu.SemaphoreType.DMA
        return pl.pallas_call(
            kernel,
            out_shape=jax.ShapeDtypeStruct((1, 1, D), A_x.dtype),
            in_specs=[hbm] * 10,
            out_specs=pl.BlockSpec(memory_space=pltpu.VMEM),
            scratch_shapes=[
                pltpu.VMEM((1, 1, D), bf16), pltpu.VMEM((D,), bf16),
                pltpu.VMEM((F,), bf16), pltpu.VMEM((D,), bf16),
                pltpu.VMEM((D, F), bf16), pltpu.VMEM((F, D), bf16),
                pltpu.VMEM((NP, D, PW), bf16),
                pltpu.VMEM((NP, PW, W), bf16), pltpu.VMEM((NP, PW, W), bf16),
                pltpu.VMEM((NP, PW, D), bf16),
                DMA((4,)), DMA((1,)), DMA((NW2,)), DMA((NP,)), DMA((NP,)), DMA((NP,)), DMA((NP,)),
            ],
            compiler_params=pltpu.CompilerParams(vmem_limit_bytes=vmem_mb << 20,
                                                 disable_bounds_checks=nobounds),
        )(A_x, kt, vt, A_wq, A_wo, B_w1, B_b1, B_w2, B_b2, gate_w)
    return fn


@jax.jit
def pallas_gated_mix__sliding_block_cached__dense_activation_gelu__decode_kernel(
    A_x, A_k_cache, A_v_cache, A_wq, A_wo, B_x, B_w1, B_b1, B_w2, B_b2, gate_w
):
    return make()(A_x, A_k_cache, A_v_cache, A_wq, A_wo, B_x, B_w1, B_b1, B_w2, B_b2, gate_w)
```

```python
import functools

import jax
import jax.numpy as jnp
from jax import lax
from jax.experimental import pallas as pl
from jax.experimental.pallas import tpu as pltpu

_HQ, _DH = 32, 192
_M = 8


class _Null:
    def __enter__(self): return None
    def __exit__(self, *a): return False


def make(NP=2, R=8, C=2048, M=_M, RQ=8, CQ=2048, R1=16, RT=48, NT=8, LA0=6, vmem_mb=100,
         compute=True, scopes=False, nobounds=False, U=1, mode="heads", split_issue=False):
    def fn(A_x, A_k_cache, A_v_cache, A_wq, A_wo, B_x, B_w1, B_b1, B_w2, B_b2, gate_w):
        del B_x
        _, _, D = A_x.shape
        _, Hkv, Sk, Dh = A_k_cache.shape
        assert Hkv == _HQ and Dh == _DH
        F = B_w1.shape[1]
        W = min(4096, max(256, Sk // 4))
        PW = 2 * Dh
        NPAIR = _HQ // 2
        HD = _HQ * Dh
        scale = Dh ** -0.5
        f32, bf16 = jnp.float32, jnp.bfloat16
        NC = W // C
        NR = PW // R
        NKV = NR * NC
        NF = F // PW
        NTAIL = NPAIR + NF
        NTP = PW // RT
        scope = (lambda n: jax.named_scope(n)) if scopes else (lambda n: _Null())

        def kernel(x_hbm, kt_hbm, vt_hbm, wq_hbm, wo_hbm, w1_hbm, b1_hbm, w2_hbm, b2_hbm, g_hbm,
                   o_ref,
                   xs, gs, b1s, b2s, w1s, wqs, kb, vb, tb, lhs,
                   sem_small, sem_w1, sem_wq, sem_k, sem_v, sem_t):

            def loop(n, f):
                if n <= 0:
                    return
                lax.fori_loop(0, n, lambda i, c: (f(i), c)[1], 0, unroll=U)

            def start_2d(hbm, buf, sem, rows, cols, r_src, c_src, nrows, ncols):
                nr, nc = nrows // rows // 2, ncols // cols

                def piece(i):
                    r, c = i // nc, i % nc
                    c0 = pl.multiple_of(c * cols, 128)
                    cs = pl.multiple_of(c_src + c * cols, 128)
                    for t in range(2):
                        r0 = pl.multiple_of(r * rows + t * (nrows // 2), 8)
                        rs = pl.multiple_of(r_src + r * rows + t * (nrows // 2), 8)
                        pltpu.make_async_copy(hbm.at[pl.ds(rs, rows), pl.ds(cs, cols)],
                                              buf.at[pl.ds(r0, rows), pl.ds(c0, cols)], sem).start(priority=t)
                loop(nr * nc, piece)

            def start_pair(j, slot):
                start_2d(kt_hbm, kb.at[slot], sem_k.at[slot], R, C, j * PW, Sk - W, PW, W)
                start_2d(vt_hbm, vb.at[slot], sem_v.at[slot], R, C, j * PW, Sk - W, PW, W)

            def start_tail(c, slot):
                @pl.when(c < NPAIR)
                def _():
                    start_2d(wo_hbm, tb.at[slot], sem_t.at[slot], RT, D, c * PW, 0, PW, D)

                @pl.when(c >= NPAIR)
                def _():
                    start_2d(w2_hbm, tb.at[slot], sem_t.at[slot], RT, D, (c - NPAIR) * PW, 0, PW, D)

            def wait_all(buf, sem):
                pltpu.make_async_copy(buf, buf, sem).wait()

            small = [pltpu.make_async_copy(x_hbm, xs, sem_small.at[0]),
                     pltpu.make_async_copy(g_hbm, gs, sem_small.at[1]),
                     pltpu.make_async_copy(b1_hbm, b1s, sem_small.at[2]),
                     pltpu.make_async_copy(b2_hbm, b2s, sem_small.at[3])]
            with scope("pro_issue"):
                for i, cp in enumerate(small):
                    cp.start(priority=i % 2)
                start_2d(w1_hbm, w1s, sem_w1.at[0], R1, F, 0, 0, D, F)
                start_2d(wq_hbm, wqs, sem_wq.at[0], RQ, CQ, 0, 0, D, HD)
                start_pair(0, 0)

            row = jax.lax.broadcasted_iota(jnp.int32, (M, PW), 0)
            col = jax.lax.broadcasted_iota(jnp.int32, (M, PW), 1)
            diag = ((row == 0) & (col < Dh)) | ((row == 1) & (col >= Dh))

            with scope("pro_compute"):
                for cp in small:
                    cp.wait()
                xv = xs[0].astype(f32)
                g = jax.nn.sigmoid(jnp.sum(xv * gs[...].astype(f32).reshape(1, D), axis=-1, keepdims=True))
                x8 = jnp.broadcast_to(xv, (M, D)).astype(bf16)

                wait_all(w1s, sem_w1.at[0])
                if compute:
                    h = jnp.dot(x8, w1s[...], preferred_element_type=f32) + b1s[...].astype(f32).reshape(1, F)
                    h = jax.nn.gelu(h, approximate=True) * (1.0 - g)
                    for i in range(NF):
                        lhs[NPAIR + i] = jnp.where(row == 0, h[:, i * PW:(i + 1) * PW], 0.0)
                else:
                    for i in range(NTAIL):
                        lhs[i] = jnp.zeros((M, PW), f32)

            with scope("pro_issue2"):
                for j in range(1, NP):
                    start_pair(j, j)
                wait_all(wqs, sem_wq.at[0])

            def body(j, carry):
                slot = j % NP
                with scope("waitK"):
                    wait_all(kb.at[slot], sem_k.at[slot])
                if compute:
                    with scope("QK"):
                        wq_j = wqs[:, pl.ds(pl.multiple_of(j * PW, 128), PW)]
                        q = jnp.dot(x8, wq_j, preferred_element_type=f32)
                        qd = jnp.where(diag, q, 0.0).astype(bf16)
                        s = jnp.dot(qd, kb[slot], preferred_element_type=f32) * scale
                        m = jnp.max(s, axis=-1, keepdims=True)
                        p = jnp.exp(s - m)
                        l = jnp.sum(p, axis=-1, keepdims=True)
                        pb = p.astype(bf16)
                if split_issue:
                    with scope("issueK"):
                        @pl.when(j + NP < NPAIR)
                        def _():
                            start_2d(kt_hbm, kb.at[slot], sem_k.at[slot], R, C, (j + NP) * PW, Sk - W, PW, W)
                with scope("waitV"):
                    wait_all(vb.at[slot], sem_v.at[slot])
                if compute:
                    with scope("PV"):
                        o = jax.lax.dot_general(pb, vb[slot], (((1,), (1,)), ((), ())),
                                                preferred_element_type=f32)
                        lhs[j] = jnp.where(diag, o * (g / l), 0.0)

                with scope("issue"):
                    @pl.when(j + NP < NPAIR)
                    def _():
                        if split_issue:
                            start_2d(vt_hbm, vb.at[slot], sem_v.at[slot], R, C, (j + NP) * PW, Sk - W, PW, W)
                        else:
                            start_pair(j + NP, slot)

                    @pl.when(j + NP == NPAIR)
                    def _():
                        for c in range(LA0):
                            start_tail(c, c % NT)
                return carry

            with scope("mainloop"):
                jax.lax.fori_loop(0, NPAIR, body, 0)

            with scope("tail_issue"):
                for c in range(LA0, NT - 1):
                    start_tail(c, c % NT)

            def tail_body(c, acc):
                slot = c % NT

                @pl.when(c + NT - 1 < NTAIL)
                def _():
                    start_tail(c + NT - 1, (c + NT - 1) % NT)
                with scope("waitT"):
                    wait_all(tb.at[slot], sem_t.at[slot])
                if compute:
                    acc = acc + jnp.dot(lhs[c].astype(bf16), tb[slot], preferred_element_type=f32)
                return acc

            with scope("tail"):
                acc = jax.lax.fori_loop(0, NTAIL, tail_body, jnp.zeros((M, D), f32))
            with scope("final"):
                res = jnp.sum(acc, axis=0, keepdims=True) + (1.0 - g) * b2s[...].astype(f32).reshape(1, D)
                o_ref[0] = res.astype(o_ref.dtype)

        kt = jnp.transpose(A_k_cache, (0, 1, 3, 2)).reshape(Hkv * Dh, Sk)
        vt = jnp.transpose(A_v_cache, (0, 1, 3, 2)).reshape(Hkv * Dh, Sk)
        hbm = pl.BlockSpec(memory_space=pl.ANY)
        DMA = pltpu.SemaphoreType.DMA
        return pl.pallas_call(
            kernel,
            out_shape=jax.ShapeDtypeStruct((1, 1, D), A_x.dtype),
            in_specs=[hbm] * 10,
            out_specs=pl.BlockSpec(memory_space=pltpu.VMEM),
            scratch_shapes=[
                pltpu.VMEM((1, 1, D), bf16), pltpu.VMEM((D,), bf16),
                pltpu.VMEM((F,), bf16), pltpu.VMEM((D,), bf16),
                pltpu.VMEM((D, F), bf16), pltpu.VMEM((D, HD), bf16),
                pltpu.VMEM((NP, PW, W), bf16), pltpu.VMEM((NP, PW, W), bf16),
                pltpu.VMEM((NT, PW, D), bf16),
                pltpu.VMEM((NTAIL, M, PW), f32),
                DMA((4,)), DMA((1,)), DMA((1,)), DMA((NP,)), DMA((NP,)), DMA((NT,)),
            ],
            compiler_params=pltpu.CompilerParams(vmem_limit_bytes=vmem_mb << 20,
                                                 disable_bounds_checks=nobounds),
        )(A_x, kt, vt, A_wq, A_wo, B_w1, B_b1, B_w2, B_b2, gate_w)
    return fn


@jax.jit
def pallas_gated_mix__sliding_block_cached__dense_activation_gelu__decode_kernel(
    A_x, A_k_cache, A_v_cache, A_wq, A_wo, B_x, B_w1, B_b1, B_w2, B_b2, gate_w
):
    return make()(A_x, A_k_cache, A_v_cache, A_wq, A_wo, B_x, B_w1, B_b1, B_w2, B_b2, gate_w)
```

```python
import functools

import jax
import jax.numpy as jnp
from jax import lax
from jax.experimental import pallas as pl
from jax.experimental.pallas import tpu as pltpu

_HQ, _DH = 32, 192
_M = 8


class _Null:
    def __enter__(self): return None
    def __exit__(self, *a): return False


def _tile_view(w):
    R, C = w.shape
    return w.reshape(R // 8, 8, C // 128, 128).transpose(0, 2, 1, 3).reshape((R // 8) * (C // 128), 8, 128)


def make(NP=2, M=_M, R1=16, vmem_mb=100, compute=True, scopes=False, U=1,
         SQ=8, SO=8, NW2=2, OC=1024, skip="", small_first=True):
    def fn(A_x, A_k_cache, A_v_cache, A_wq, A_wo, B_x, B_w1, B_b1, B_w2, B_b2, gate_w):
        del B_x
        _, _, D = A_x.shape
        _, Hkv, Sk, Dh = A_k_cache.shape
        assert Hkv == _HQ and Dh == _DH
        F = B_w1.shape[1]
        W = min(4096, max(256, Sk // 4))
        PW = 2 * Dh
        NPAIR = _HQ // 2
        HD = _HQ * Dh
        scale = Dh ** -0.5
        f32, bf16 = jnp.float32, jnp.bfloat16
        NCT = D // 128
        PC = 2048
        scope = (lambda n: jax.named_scope(n)) if scopes else (lambda n: _Null())

        def perm(i, n, s):
            if s == 1:
                return i
            p = n + 1
            while any(p % d == 0 for d in range(2, p)):
                p += 1
            assert p == n + 1 and p % s != 0
            return (s * (i + 1)) % p - 1

        for n_, s_ in ((60, SQ), (60, SO)):
            assert sorted(perm(i, n_, s_) for i in range(n_)) == list(range(n_))

        def kernel(x_hbm, kt_hbm, vt_hbm, wq_hbm, wo_hbm, w1_hbm, b1_hbm, w2_hbm, b2_hbm, g_hbm,
                   o_ref,
                   xs, gs, b1s, b2s, w1s, wqs, kb, vb, wos, w2s, lhs,
                   sem_small, sem_w1, sem_wq, sem_k, sem_v, sem_wo, sem_w2):

            def loop(n, f):
                if n <= 0:
                    return
                lax.fori_loop(0, n, lambda i, c: (f(i), c)[1], 0, unroll=U)

            def start_w1():
                n = D // R1 // 2

                def piece(i):
                    for t in range(2):
                        r0 = pl.multiple_of((i + t * n) * R1, 8)
                        pltpu.make_async_copy(w1_hbm.at[pl.ds(r0, R1), :], w1s.at[pl.ds(r0, R1), :],
                                              sem_w1.at[0]).start(priority=t)
                loop(n, piece)

            def start_wq():
                ppr = HD // PC
                nb = (D // 8) * ppr // 2 // 2

                def block(i):
                    for u in range(2):
                        for t in range(2):
                            k = 2 * (perm(i, nb, SQ) + t * nb) + u
                            r0 = pl.multiple_of((k // ppr) * 8, 8)
                            c0 = pl.multiple_of((k % ppr) * PC, 128)
                            pltpu.make_async_copy(wq_hbm.at[pl.ds(r0, 8), pl.ds(c0, PC)],
                                                  wqs.at[pl.ds(r0, 8), pl.ds(c0, PC)],
                                                  sem_wq.at[0]).start(priority=t)
                loop(nb, block)

            def start_window(hbm, buf, sem, j):
                def block(i):
                    for u in range(W // PC):
                        for t in range(2):
                            r0 = pl.multiple_of(i * 8 + t * Dh, 8)
                            rs = pl.multiple_of(j * PW + i * 8 + t * Dh, 8)
                            pltpu.make_async_copy(hbm.at[pl.ds(rs, 8), pl.ds(Sk - W + u * PC, PC)],
                                                  buf.at[pl.ds(r0, 8), pl.ds(u * PC, PC)], sem).start(priority=t)
                loop(Dh // 8, block)

            def start_pair(j, slot):
                start_window(kt_hbm, kb.at[slot], sem_k.at[slot], j)
                start_window(vt_hbm, vb.at[slot], sem_v.at[slot], j)

            def start_wo():
                nb = wo_hbm.shape[0] // 32 // 2

                def block(i):
                    for u in range(2):
                        for t in range(2):
                            t0 = pl.multiple_of(32 * (perm(i, nb, SO) + t * nb) + 16 * u, 16)
                            pltpu.make_async_copy(wo_hbm.at[pl.ds(t0, 16)], wos.at[pl.ds(t0, 16)],
                                                  sem_wo.at[0]).start(priority=t)
                loop(nb, block)

            W2T = w2_hbm.shape[0] // NW2

            def start_w2():
                n = W2T // 16 // 2

                def piece(i):
                    c, k = i // n, i % n
                    for t in range(2):
                        t0 = pl.multiple_of(c * W2T + (k + t * n) * 16, 16)
                        pltpu.make_async_copy(w2_hbm.at[pl.ds(t0, 16)], w2s.at[pl.ds(t0, 16)],
                                              sem_w2.at[c]).start(priority=t)
                loop(NW2 * n, piece)

            def wait_all(buf, sem):
                pltpu.make_async_copy(buf, buf, sem).wait()

            def rows_times_tiles(lhs_bf, buf, rg0, nrg):
                outs = []
                for ct in range(NCT):
                    rhs = buf[pl.ds(rg0 * NCT + ct, nrg, stride=NCT)].reshape(nrg * 8, 128)
                    outs.append(jnp.dot(lhs_bf, rhs, preferred_element_type=f32))
                return jnp.concatenate(outs, axis=1)

            small = [pltpu.make_async_copy(x_hbm, xs, sem_small.at[0]),
                     pltpu.make_async_copy(g_hbm, gs, sem_small.at[1]),
                     pltpu.make_async_copy(b1_hbm, b1s, sem_small.at[2]),
                     pltpu.make_async_copy(b2_hbm, b2s, sem_small.at[3])]
            with scope("pro_issue"):
                if small_first:
                    for i, cp in enumerate(small):
                        cp.start(priority=i % 2)
                start_wq()
                if not small_first:
                    for i, cp in enumerate(small):
                        cp.start(priority=i % 2)
                start_w1()
                start_pair(0, 0)

            row = jax.lax.broadcasted_iota(jnp.int32, (M, PW), 0)
            col = jax.lax.broadcasted_iota(jnp.int32, (M, PW), 1)
            diag = ((row == 0) & (col < Dh)) | ((row == 1) & (col >= Dh))

            with scope("pro_compute"):
                for cp in small:
                    cp.wait()
                xv = xs[0].astype(f32)
                g = jax.nn.sigmoid(jnp.sum(xv * gs[...].astype(f32).reshape(1, D), axis=-1, keepdims=True))
                x8 = jnp.broadcast_to(xv, (M, D)).astype(bf16)

                wait_all(w1s, sem_w1.at[0])
                if compute:
                    h = jnp.dot(x8, w1s[...], preferred_element_type=f32) + b1s[...].astype(f32).reshape(1, F)
                    h = jax.nn.gelu(h, approximate=True) * (1.0 - g)
                    rowf = jax.lax.broadcasted_iota(jnp.int32, (M, F), 0)
                    hb = jnp.where(rowf == 0, h, 0.0).astype(bf16)
                else:
                    hb = jnp.zeros((M, F), bf16)
                    lhs[...] = jnp.zeros((M, HD), f32)
                wait_all(wqs, sem_wq.at[0])

            with scope("pro_issue2"):
                for j in range(1, NP):
                    start_pair(j, j)

            def body(j, carry):
                slot = j % NP
                with scope("waitK"):
                    wait_all(kb.at[slot], sem_k.at[slot])
                if compute:
                    with scope("QK"):
                        wq_j = wqs[:, pl.ds(pl.multiple_of(j * PW, 128), PW)]
                        q = jnp.dot(x8, wq_j, preferred_element_type=f32)
                        qd = jnp.where(diag, q, 0.0).astype(bf16)
                        s = jnp.dot(qd, kb[slot], preferred_element_type=f32) * scale
                        m = jnp.max(s, axis=-1, keepdims=True)
                        p = jnp.exp(s - m)
                        l = jnp.sum(p, axis=-1, keepdims=True)
                        pb = p.astype(bf16)
                with scope("waitV"):
                    wait_all(vb.at[slot], sem_v.at[slot])
                if compute:
                    with scope("PV"):
                        o = jax.lax.dot_general(pb, vb[slot], (((1,), (1,)), ((), ())),
                                                preferred_element_type=f32)
                        lhs[:, pl.ds(pl.multiple_of(j * PW, 128), PW)] = jnp.where(diag, o * (g / l), 0.0)

                with scope("issue"):
                    @pl.when(j + NP < NPAIR)
                    def _():
                        start_pair(j + NP, slot)

                    @pl.when(j + NP == NPAIR)
                    def _():
                        start_wo()
                        start_w2()
                return carry

            with scope("mainloop"):
                jax.lax.fori_loop(0, NPAIR, body, 0)

            with scope("waitWo"):
                wait_all(wos, sem_wo.at[0])
            acc = jnp.zeros((M, D), f32)
            with scope("wo"):
                if compute:
                    for c in range(HD // OC):
                        l_c = lhs[:, c * OC:(c + 1) * OC].astype(bf16)
                        acc = acc + rows_times_tiles(l_c, wos, c * (OC // 8), OC // 8)
            with scope("w2"):
                for c in range(NW2):
                    with scope("waitW2"):
                        wait_all(w2s.at[pl.ds(c * W2T, W2T)], sem_w2.at[c])
                    if compute:
                        nrg = W2T // NCT
                        acc = acc + rows_times_tiles(hb[:, c * nrg * 8:(c + 1) * nrg * 8], w2s, c * nrg, nrg)
            with scope("final"):
                res = jnp.sum(acc, axis=0, keepdims=True) + (1.0 - g) * b2s[...].astype(f32).reshape(1, D)
                o_ref[0] = res.astype(o_ref.dtype)

        kt = jnp.transpose(A_k_cache, (0, 1, 3, 2)).reshape(Hkv * Dh, Sk)
        vt = jnp.transpose(A_v_cache, (0, 1, 3, 2)).reshape(Hkv * Dh, Sk)
        wo_t, w2_t = _tile_view(A_wo), _tile_view(B_w2)
        hbm = pl.BlockSpec(memory_space=pl.ANY)
        DMA = pltpu.SemaphoreType.DMA
        return pl.pallas_call(
            kernel,
            out_shape=jax.ShapeDtypeStruct((1, 1, D), A_x.dtype),
            in_specs=[hbm] * 10,
            out_specs=pl.BlockSpec(memory_space=pltpu.VMEM),
            scratch_shapes=[
                pltpu.VMEM((1, 1, D), bf16), pltpu.VMEM((D,), bf16),
                pltpu.VMEM((F,), bf16), pltpu.VMEM((D,), bf16),
                pltpu.VMEM((D, F), bf16), pltpu.VMEM((D, HD), bf16),
                pltpu.VMEM((NP, PW, W), bf16), pltpu.VMEM((NP, PW, W), bf16),
                pltpu.VMEM(wo_t.shape, bf16), pltpu.VMEM(w2_t.shape, bf16),
                pltpu.VMEM((M, HD), f32),
                DMA((4,)), DMA((1,)), DMA((1,)), DMA((NP,)), DMA((NP,)), DMA((1,)), DMA((NW2,)),
            ],
            compiler_params=pltpu.CompilerParams(vmem_limit_bytes=vmem_mb << 20),
        )(A_x, kt, vt, A_wq, wo_t, B_w1, B_b1, w2_t, B_b2, gate_w)
    return fn


@jax.jit
def pallas_gated_mix__sliding_block_cached__dense_activation_gelu__decode_kernel(
    A_x, A_k_cache, A_v_cache, A_wq, A_wo, B_x, B_w1, B_b1, B_w2, B_b2, gate_w
):
    return make()(A_x, A_k_cache, A_v_cache, A_wq, A_wo, B_x, B_w1, B_b1, B_w2, B_b2, gate_w)
```

```python
import functools

import jax
import jax.numpy as jnp
from jax import lax
from jax.experimental import pallas as pl
from jax.experimental.pallas import tpu as pltpu

_HQ, _DH = 32, 192
_M = 8


class _Null:
    def __enter__(self): return None
    def __exit__(self, *a): return False


def _tile_view(w):
    R, C = w.shape
    return w.reshape(R // 8, 8, C // 128, 128).transpose(0, 2, 1, 3).reshape((R // 8) * (C // 128), 8, 128)


def make(NP=2, M=_M, R1=16, vmem_mb=100, compute=True, scopes=False, U=1,
         SQ=8, SO=8, W2C=(640, 240, 80), OC=1024, skip="", small_first=True, NG=3, NAG=1):
    def fn(A_x, A_k_cache, A_v_cache, A_wq, A_wo, B_x, B_w1, B_b1, B_w2, B_b2, gate_w):
        del B_x
        _, _, D = A_x.shape
        _, Hkv, Sk, Dh = A_k_cache.shape
        assert Hkv == _HQ and Dh == _DH
        F = B_w1.shape[1]
        W = min(4096, max(256, Sk // 4))
        PW = 2 * Dh
        NPAIR = _HQ // 2
        HD = _HQ * Dh
        scale = Dh ** -0.5
        f32, bf16 = jnp.float32, jnp.bfloat16
        NCT = D // 128
        PC = 2048
        scope = (lambda n: jax.named_scope(n)) if scopes else (lambda n: _Null())

        def perm(i, n, s):
            if s == 1:
                return i
            return (s * (i + 1)) % (n + 1) - 1

        for n_, s_ in ((60, SQ), (60 // NG, SO)):
            assert sorted(perm(i, n_, s_) for i in range(n_)) == list(range(n_))

        def kernel(x_hbm, kt_hbm, vt_hbm, wq_hbm, wo_hbm, w1_hbm, b1_hbm, w2_hbm, b2_hbm, g_hbm,
                   o_ref,
                   xs, gs, b1s, b2s, w1s, wqs, kb, vb, wos, w2s, lhs,
                   sem_small, sem_w1, sem_wq, sem_k, sem_v, sem_wo, sem_w2):

            def loop(n, f):
                if n <= 0:
                    return
                lax.fori_loop(0, n, lambda i, c: (f(i), c)[1], 0, unroll=U)

            def start_w1():
                n = D // R1 // 2

                def piece(i):
                    for t in range(2):
                        r0 = pl.multiple_of((i + t * n) * R1, 8)
                        pltpu.make_async_copy(w1_hbm.at[pl.ds(r0, R1), :], w1s.at[pl.ds(r0, R1), :],
                                              sem_w1.at[0]).start(priority=t)
                loop(n, piece)

            def start_wq():
                ppr = HD // PC
                nb = (D // 8) * ppr // 2 // 2

                def block(i):
                    for u in range(2):
                        for t in range(2):
                            k = 2 * (perm(i, nb, SQ) + t * nb) + u
                            r0 = pl.multiple_of((k // ppr) * 8, 8)
                            c0 = pl.multiple_of((k % ppr) * PC, 128)
                            pltpu.make_async_copy(wq_hbm.at[pl.ds(r0, 8), pl.ds(c0, PC)],
                                                  wqs.at[pl.ds(r0, 8), pl.ds(c0, PC)],
                                                  sem_wq.at[0]).start(priority=t)
                loop(nb, block)

            def start_window(hbm, buf, sem, j):
                def block(i):
                    for u in range(W // PC):
                        for t in range(2):
                            r0 = pl.multiple_of(i * 8 + t * Dh, 8)
                            rs = pl.multiple_of(j * PW + i * 8 + t * Dh, 8)
                            pltpu.make_async_copy(hbm.at[pl.ds(rs, 8), pl.ds(Sk - W + u * PC, PC)],
                                                  buf.at[pl.ds(r0, 8), pl.ds(u * PC, PC)], sem).start(priority=t)
                loop(Dh // 8, block)

            def start_pair(j, slot):
                start_window(kt_hbm, kb.at[slot], sem_k.at[slot], j)
                start_window(vt_hbm, vb.at[slot], sem_v.at[slot], j)

            WOB = wo_hbm.shape[0] // 32 // 2
            GB = WOB // NG

            def start_wo(g):
                def block(i):
                    for u in range(2):
                        for t in range(2):
                            t0 = pl.multiple_of(32 * (perm(i, GB, SO) + g * GB + t * WOB) + 16 * u, 16)
                            pltpu.make_async_copy(wo_hbm.at[pl.ds(t0, 16)], wos.at[pl.ds(t0, 16)],
                                                  sem_wo.at[g]).start(priority=t)
                loop(GB, block)

            W2OFF = [sum(W2C[:c]) for c in range(len(W2C))]
            assert sum(W2C) == w2_hbm.shape[0] and all(n % 80 == 0 for n in W2C)

            def start_w2():
                for c, (off, ntile) in enumerate(zip(W2OFF, W2C)):
                    half = ntile // 2
                    P = max(p for p in (16, 20, 10, 8) if half % p == 0)

                    def piece(k, off=off, half=half, P=P, c=c):
                        for t in range(2):
                            t0 = pl.multiple_of(off + t * half + k * P, 2)
                            pltpu.make_async_copy(w2_hbm.at[pl.ds(t0, P)], w2s.at[pl.ds(t0, P)],
                                                  sem_w2.at[c]).start(priority=t)
                    loop(half // P, piece)

            def wait_all(buf, sem):
                pltpu.make_async_copy(buf, buf, sem).wait()

            def rows_times_tiles(lhs_bf, buf, rg0, nrg):
                outs = []
                for ct in range(NCT):
                    rhs = buf[pl.ds(rg0 * NCT + ct, nrg, stride=NCT)].reshape(nrg * 8, 128)
                    outs.append(jnp.dot(lhs_bf, rhs, preferred_element_type=f32))
                return jnp.concatenate(outs, axis=1)

            small = [pltpu.make_async_copy(x_hbm, xs, sem_small.at[0]),
                     pltpu.make_async_copy(g_hbm, gs, sem_small.at[1]),
                     pltpu.make_async_copy(b1_hbm, b1s, sem_small.at[2]),
                     pltpu.make_async_copy(b2_hbm, b2s, sem_small.at[3])]
            with scope("pro_issue"):
                if small_first:
                    for i, cp in enumerate(small):
                        cp.start(priority=i % 2)
                start_wq()
                if not small_first:
                    for i, cp in enumerate(small):
                        cp.start(priority=i % 2)
                start_w1()
                start_pair(0, 0)

            row = jax.lax.broadcasted_iota(jnp.int32, (M, PW), 0)
            col = jax.lax.broadcasted_iota(jnp.int32, (M, PW), 1)
            diag = ((row == 0) & (col < Dh)) | ((row == 1) & (col >= Dh))

            with scope("pro_compute"):
                for cp in small:
                    cp.wait()
                xv = xs[0].astype(f32)
                g = jax.nn.sigmoid(jnp.sum(xv * gs[...].astype(f32).reshape(1, D), axis=-1, keepdims=True))
                x8 = jnp.broadcast_to(xv, (M, D)).astype(bf16)

                wait_all(w1s, sem_w1.at[0])
                if compute:
                    h = jnp.dot(x8, w1s[...], preferred_element_type=f32) + b1s[...].astype(f32).reshape(1, F)
                    h = jax.nn.gelu(h, approximate=True) * (1.0 - g)
                    rowf = jax.lax.broadcasted_iota(jnp.int32, (M, F), 0)
                    hb = jnp.where(rowf == 0, h, 0.0).astype(bf16)
                else:
                    hb = jnp.zeros((M, F), bf16)
                    lhs[...] = jnp.zeros((M, HD), f32)
                wait_all(wqs, sem_wq.at[0])

            with scope("pro_issue2"):
                for j in range(1, NP):
                    start_pair(j, j)

            def body(j, carry):
                slot = j % NP
                with scope("waitK"):
                    wait_all(kb.at[slot], sem_k.at[slot])
                if compute:
                    with scope("QK"):
                        wq_j = wqs[:, pl.ds(pl.multiple_of(j * PW, 128), PW)]
                        q = jnp.dot(x8, wq_j, preferred_element_type=f32)
                        qd = jnp.where(diag, q, 0.0).astype(bf16)
                        s = jnp.dot(qd, kb[slot], preferred_element_type=f32) * scale
                        m = jnp.max(s, axis=-1, keepdims=True)
                        p = jnp.exp(s - m)
                        l = jnp.sum(p, axis=-1, keepdims=True)
                        pb = p.astype(bf16)
                with scope("waitV"):
                    wait_all(vb.at[slot], sem_v.at[slot])
                if compute:
                    with scope("PV"):
                        o = jax.lax.dot_general(pb, vb[slot], (((1,), (1,)), ((), ())),
                                                preferred_element_type=f32)
                        lhs[:, pl.ds(pl.multiple_of(j * PW, 128), PW)] = jnp.where(diag, o * (g / l), 0.0)

                with scope("issue"):
                    @pl.when(j + NP < NPAIR)
                    def _():
                        start_pair(j + NP, slot)

                    with scope("issueA"):
                      @pl.when(j + NP == NPAIR)
                      def _():
                        for g_ in range(NAG):
                            start_wo(g_)
                return carry

            with scope("mainloop"):
                jax.lax.fori_loop(0, NPAIR, body, 0)

            with scope("tail_issue"):
                for g_ in range(NAG, NG):
                    start_wo(g_)
                start_w2()
            acc = jnp.zeros((M, D), f32)
            GR = GB * 32 // NCT
            for g_ in range(NG):
                with scope("waitWo"):
                    for t in range(2):
                        wait_all(wos.at[pl.ds((g_ * GB + t * WOB) * 32, GB * 32)], sem_wo.at[g_])
                with scope("wo"):
                    if compute:
                        for t in range(2):
                            rg0 = (g_ * GB + t * WOB) * 32 // NCT
                            l_c = lhs[:, rg0 * 8:(rg0 + GR) * 8].astype(bf16)
                            acc = acc + rows_times_tiles(l_c, wos, rg0, GR)
            with scope("w2"):
                for c, (off, ntile) in enumerate(zip(W2OFF, W2C)):
                    with scope("waitW2"):
                        wait_all(w2s.at[pl.ds(off, ntile)], sem_w2.at[c])
                    if compute:
                        rg0, nrg = off // NCT, ntile // NCT
                        acc = acc + rows_times_tiles(hb[:, rg0 * 8:(rg0 + nrg) * 8], w2s, rg0, nrg)
            with scope("final"):
                res = jnp.sum(acc, axis=0, keepdims=True) + (1.0 - g) * b2s[...].astype(f32).reshape(1, D)
                o_ref[0] = res.astype(o_ref.dtype)

        kt = jnp.transpose(A_k_cache, (0, 1, 3, 2)).reshape(Hkv * Dh, Sk)
        vt = jnp.transpose(A_v_cache, (0, 1, 3, 2)).reshape(Hkv * Dh, Sk)
        wo_t, w2_t = _tile_view(A_wo), _tile_view(B_w2)
        hbm = pl.BlockSpec(memory_space=pl.ANY)
        DMA = pltpu.SemaphoreType.DMA
        return pl.pallas_call(
            kernel,
            out_shape=jax.ShapeDtypeStruct((1, 1, D), A_x.dtype),
            in_specs=[hbm] * 10,
            out_specs=pl.BlockSpec(memory_space=pltpu.VMEM),
            scratch_shapes=[
                pltpu.VMEM((1, 1, D), bf16), pltpu.VMEM((D,), bf16),
                pltpu.VMEM((F,), bf16), pltpu.VMEM((D,), bf16),
                pltpu.VMEM((D, F), bf16), pltpu.VMEM((D, HD), bf16),
                pltpu.VMEM((NP, PW, W), bf16), pltpu.VMEM((NP, PW, W), bf16),
                pltpu.VMEM(wo_t.shape, bf16), pltpu.VMEM(w2_t.shape, bf16),
                pltpu.VMEM((M, HD), f32),
                DMA((4,)), DMA((1,)), DMA((1,)), DMA((NP,)), DMA((NP,)), DMA((NG,)), DMA((len(W2C),)),
            ],
            compiler_params=pltpu.CompilerParams(vmem_limit_bytes=vmem_mb << 20),
        )(A_x, kt, vt, A_wq, wo_t, B_w1, B_b1, w2_t, B_b2, gate_w)
    return fn


@jax.jit
def pallas_gated_mix__sliding_block_cached__dense_activation_gelu__decode_kernel(
    A_x, A_k_cache, A_v_cache, A_wq, A_wo, B_x, B_w1, B_b1, B_w2, B_b2, gate_w
):
    return make()(A_x, A_k_cache, A_v_cache, A_wq, A_wo, B_x, B_w1, B_b1, B_w2, B_b2, gate_w)
```

```python
import functools

import jax
import jax.numpy as jnp
from jax import lax
from jax.experimental import pallas as pl
from jax.experimental.pallas import tpu as pltpu

_HQ, _DH = 32, 192
_M = 8


class _Null:
    def __enter__(self): return None
    def __exit__(self, *a): return False


def _tile_view(w):
    R, C = w.shape
    return w.reshape(R // 8, 8, C // 128, 128).transpose(0, 2, 1, 3).reshape((R // 8) * (C // 128), 8, 128)


def make(NP=2, M=_M, R1=16, vmem_mb=100, compute=True, scopes=False, U=1,
         SQ=8, SO=8, W2C=(640, 240, 80), OC=1024, skip="", small_first=True, NG=3, NAG=2, KCUT=(2048, 0), VCUT=(3072, 1), WSH=1):
    def fn(A_x, A_k_cache, A_v_cache, A_wq, A_wo, B_x, B_w1, B_b1, B_w2, B_b2, gate_w):
        del B_x
        _, _, D = A_x.shape
        _, Hkv, Sk, Dh = A_k_cache.shape
        assert Hkv == _HQ and Dh == _DH
        F = B_w1.shape[1]
        W = min(4096, max(256, Sk // 4))
        PW = 2 * Dh
        NPAIR = _HQ // 2
        HD = _HQ * Dh
        scale = Dh ** -0.5
        f32, bf16 = jnp.float32, jnp.bfloat16
        NCT = D // 128
        PC = 2048
        scope = (lambda n: jax.named_scope(n)) if scopes else (lambda n: _Null())

        def perm(i, n, s):
            if s == 1:
                return i
            return (s * (i + 1)) % (n + 1) - 1

        for n_, s_ in ((60, SQ), (60 // NG, SO)):
            assert sorted(perm(i, n_, s_) for i in range(n_)) == list(range(n_))

        def kernel(x_hbm, kt_hbm, vt_hbm, wq_hbm, wo_hbm, w1_hbm, b1_hbm, w2_hbm, b2_hbm, g_hbm,
                   o_ref,
                   xs, gs, b1s, b2s, w1s, wqs, kb, vb, wos, w2s, lhs,
                   sem_small, sem_w1, sem_wq, sem_k, sem_v, sem_wo, sem_w2):

            def loop(n, f):
                if n <= 0:
                    return
                lax.fori_loop(0, n, lambda i, c: (f(i), c)[1], 0, unroll=U)

            def start_w1():
                n = D // R1 // 2

                def piece(i):
                    for t in range(2):
                        r0 = pl.multiple_of((i + t * n) * R1, 8)
                        pltpu.make_async_copy(w1_hbm.at[pl.ds(r0, R1), :], w1s.at[pl.ds(r0, R1), :],
                                              sem_w1.at[0]).start(priority=t)
                loop(n, piece)

            def start_wq():
                ppr = HD // PC
                nb = (D // 8) * ppr // 2 // 2

                def block(i):
                    for u in range(2):
                        for t in range(2):
                            k = lax.rem(2 * perm(i, nb, SQ) + u + WSH, 2 * nb) + t * 2 * nb
                            r0 = pl.multiple_of((k // ppr) * 8, 8)
                            c0 = pl.multiple_of((k % ppr) * PC, 128)
                            pltpu.make_async_copy(wq_hbm.at[pl.ds(r0, 8), pl.ds(c0, PC)],
                                                  wqs.at[pl.ds(r0, 8), pl.ds(c0, PC)],
                                                  sem_wq.at[0]).start(priority=t)
                loop(nb, block)

            def start_window(hbm, buf, sem, j, cut, t_lo):
                def rowgroup(i):
                    r0 = pl.multiple_of(i * 8, 8)
                    rs = pl.multiple_of(j * PW + i * 8, 8)
                    for c0, c1, t in ((0, cut, t_lo), (cut, W, 1 - t_lo)):
                        pltpu.make_async_copy(hbm.at[pl.ds(rs, 8), pl.ds(Sk - W + c0, c1 - c0)],
                                              buf.at[pl.ds(r0, 8), pl.ds(c0, c1 - c0)], sem).start(priority=t)
                loop(PW // 8, rowgroup)

            def start_pair(j, slot):
                start_window(kt_hbm, kb.at[slot], sem_k.at[slot], j, *KCUT)
                start_window(vt_hbm, vb.at[slot], sem_v.at[slot], j, *VCUT)

            WOB = wo_hbm.shape[0] // 32 // 2
            GB = WOB // NG

            def start_wo(g):
                def block(i):
                    for u in range(2):
                        for t in range(2):
                            k = lax.rem(2 * perm(i, GB, SO) + u + WSH, 2 * GB)
                            t0 = pl.multiple_of(16 * k + 32 * (g * GB + t * WOB), 16)
                            pltpu.make_async_copy(wo_hbm.at[pl.ds(t0, 16)], wos.at[pl.ds(t0, 16)],
                                                  sem_wo.at[g]).start(priority=t)
                loop(GB, block)

            W2OFF = [sum(W2C[:c]) for c in range(len(W2C))]
            assert sum(W2C) == w2_hbm.shape[0] and all(n % 80 == 0 for n in W2C)

            def start_w2():
                for c, (off, ntile) in enumerate(zip(W2OFF, W2C)):
                    half = ntile // 2
                    P = max(p for p in (16, 20, 10, 8) if half % p == 0)

                    def piece(k, off=off, half=half, P=P, c=c):
                        for t in range(2):
                            t0 = pl.multiple_of(off + t * half + k * P, 2)
                            pltpu.make_async_copy(w2_hbm.at[pl.ds(t0, P)], w2s.at[pl.ds(t0, P)],
                                                  sem_w2.at[c]).start(priority=t)
                    loop(half // P, piece)

            def wait_all(buf, sem):
                pltpu.make_async_copy(buf, buf, sem).wait()

            def rows_times_tiles(lhs_bf, buf, rg0, nrg):
                outs = []
                for ct in range(NCT):
                    rhs = buf[pl.ds(rg0 * NCT + ct, nrg, stride=NCT)].reshape(nrg * 8, 128)
                    outs.append(jnp.dot(lhs_bf, rhs, preferred_element_type=f32))
                return jnp.concatenate(outs, axis=1)

            small = [pltpu.make_async_copy(x_hbm, xs, sem_small.at[0]),
                     pltpu.make_async_copy(g_hbm, gs, sem_small.at[1]),
                     pltpu.make_async_copy(b1_hbm, b1s, sem_small.at[2]),
                     pltpu.make_async_copy(b2_hbm, b2s, sem_small.at[3])]
            with scope("pro_issue"):
                if small_first:
                    for i, cp in enumerate(small):
                        cp.start(priority=i % 2)
                start_wq()
                if not small_first:
                    for i, cp in enumerate(small):
                        cp.start(priority=i % 2)
                start_w1()
                start_pair(0, 0)

            row = jax.lax.broadcasted_iota(jnp.int32, (M, PW), 0)
            col = jax.lax.broadcasted_iota(jnp.int32, (M, PW), 1)
            diag = ((row == 0) & (col < Dh)) | ((row == 1) & (col >= Dh))

            with scope("pro_compute"):
                for cp in small:
                    cp.wait()
                xv = xs[0].astype(f32)
                g = jax.nn.sigmoid(jnp.sum(xv * gs[...].astype(f32).reshape(1, D), axis=-1, keepdims=True))
                x8 = jnp.broadcast_to(xv, (M, D)).astype(bf16)

                wait_all(w1s, sem_w1.at[0])
                if compute:
                    h = jnp.dot(x8, w1s[...], preferred_element_type=f32) + b1s[...].astype(f32).reshape(1, F)
                    h = jax.nn.gelu(h, approximate=True) * (1.0 - g)
                    rowf = jax.lax.broadcasted_iota(jnp.int32, (M, F), 0)
                    hb = jnp.where(rowf == 0, h, 0.0).astype(bf16)
                else:
                    hb = jnp.zeros((M, F), bf16)
                    lhs[...] = jnp.zeros((M, HD), f32)
                wait_all(wqs, sem_wq.at[0])

            with scope("pro_issue2"):
                for j in range(1, NP):
                    start_pair(j, j)

            def body(j, carry):
                slot = j % NP
                with scope("waitK"):
                    wait_all(kb.at[slot], sem_k.at[slot])
                if compute:
                    with scope("QK"):
                        wq_j = wqs[:, pl.ds(pl.multiple_of(j * PW, 128), PW)]
                        q = jnp.dot(x8, wq_j, preferred_element_type=f32)
                        qd = jnp.where(diag, q, 0.0).astype(bf16)
                        s = jnp.dot(qd, kb[slot], preferred_element_type=f32) * scale
                        m = jnp.max(s, axis=-1, keepdims=True)
                        p = jnp.exp(s - m)
                        l = jnp.sum(p, axis=-1, keepdims=True)
                        pb = p.astype(bf16)
                with scope("waitV"):
                    wait_all(vb.at[slot], sem_v.at[slot])
                if compute:
                    with scope("PV"):
                        o = jax.lax.dot_general(pb, vb[slot], (((1,), (1,)), ((), ())),
                                                preferred_element_type=f32)
                        lhs[:, pl.ds(pl.multiple_of(j * PW, 128), PW)] = jnp.where(diag, o * (g / l), 0.0)

                with scope("issue"):
                    @pl.when(j + NP < NPAIR)
                    def _():
                        start_pair(j + NP, slot)

                    with scope("issueA"):
                      @pl.when(j + NP == NPAIR)
                      def _():
                        for g_ in range(NAG):
                            start_wo(g_)
                return carry

            with scope("mainloop"):
                jax.lax.fori_loop(0, NPAIR, body, 0)

            with scope("tail_issue"):
                for g_ in range(NAG, NG):
                    start_wo(g_)
                start_w2()
            acc = jnp.zeros((M, D), f32)
            GR = GB * 32 // NCT
            for g_ in range(NG):
                with scope("waitWo"):
                    for t in range(2):
                        wait_all(wos.at[pl.ds((g_ * GB + t * WOB) * 32, GB * 32)], sem_wo.at[g_])
                with scope("wo"):
                    if compute:
                        for t in range(2):
                            rg0 = (g_ * GB + t * WOB) * 32 // NCT
                            l_c = lhs[:, rg0 * 8:(rg0 + GR) * 8].astype(bf16)
                            acc = acc + rows_times_tiles(l_c, wos, rg0, GR)
            with scope("w2"):
                for c, (off, ntile) in enumerate(zip(W2OFF, W2C)):
                    with scope("waitW2"):
                        wait_all(w2s.at[pl.ds(off, ntile)], sem_w2.at[c])
                    if compute:
                        rg0, nrg = off // NCT, ntile // NCT
                        acc = acc + rows_times_tiles(hb[:, rg0 * 8:(rg0 + nrg) * 8], w2s, rg0, nrg)
            with scope("final"):
                res = jnp.sum(acc, axis=0, keepdims=True) + (1.0 - g) * b2s[...].astype(f32).reshape(1, D)
                o_ref[0] = res.astype(o_ref.dtype)

        kt = jnp.transpose(A_k_cache, (0, 1, 3, 2)).reshape(Hkv * Dh, Sk)
        vt = jnp.transpose(A_v_cache, (0, 1, 3, 2)).reshape(Hkv * Dh, Sk)
        wo_t, w2_t = _tile_view(A_wo), _tile_view(B_w2)
        hbm = pl.BlockSpec(memory_space=pl.ANY)
        DMA = pltpu.SemaphoreType.DMA
        return pl.pallas_call(
            kernel,
            out_shape=jax.ShapeDtypeStruct((1, 1, D), A_x.dtype),
            in_specs=[hbm] * 10,
            out_specs=pl.BlockSpec(memory_space=pltpu.VMEM),
            scratch_shapes=[
                pltpu.VMEM((1, 1, D), bf16), pltpu.VMEM((D,), bf16),
                pltpu.VMEM((F,), bf16), pltpu.VMEM((D,), bf16),
                pltpu.VMEM((D, F), bf16), pltpu.VMEM((D, HD), bf16),
                pltpu.VMEM((NP, PW, W), bf16), pltpu.VMEM((NP, PW, W), bf16),
                pltpu.VMEM(wo_t.shape, bf16), pltpu.VMEM(w2_t.shape, bf16),
                pltpu.VMEM((M, HD), f32),
                DMA((4,)), DMA((1,)), DMA((1,)), DMA((NP,)), DMA((NP,)), DMA((NG,)), DMA((len(W2C),)),
            ],
            compiler_params=pltpu.CompilerParams(vmem_limit_bytes=vmem_mb << 20),
        )(A_x, kt, vt, A_wq, wo_t, B_w1, B_b1, w2_t, B_b2, gate_w)
    return fn


@jax.jit
def pallas_gated_mix__sliding_block_cached__dense_activation_gelu__decode_kernel(
    A_x, A_k_cache, A_v_cache, A_wq, A_wo, B_x, B_w1, B_b1, B_w2, B_b2, gate_w
):
    return make()(A_x, A_k_cache, A_v_cache, A_wq, A_wo, B_x, B_w1, B_b1, B_w2, B_b2, gate_w)
```

```python
import jax
import jax.numpy as jnp
from jax import lax
from jax.experimental import pallas as pl
from jax.experimental.pallas import tpu as pltpu

_HQ, _DH = 32, 192
_M = 8
_NP = 2
_TILE_BLK = 32
_STRIDE = 8
_K_CUT = (2048, 0)
_V_CUT = (3072, 1)
_BLK_PHASE = 1
_WO_GROUPS = 3
_WO_EARLY = 2
_W2_CHUNKS = (640, 240, 80)
_W1_ROWS = 16


def _tile_view(w):
    R, C = w.shape
    return w.reshape(R // 8, 8, C // 128, 128).transpose(0, 2, 1, 3).reshape((R // 8) * (C // 128), 8, 128)


def _perm(i, n):
    return (_STRIDE * (i + 1)) % (n + 1) - 1


def _check_perm(n):
    assert sorted(_perm(i, n) for i in range(n)) == list(range(n)), n


def _loop(n, f):
    lax.fori_loop(0, n, lambda i, c: (f(i), c)[1], 0)


def _wait_filled(buf, sem):
    pltpu.make_async_copy(buf, buf, sem).wait()


@jax.jit
def pallas_gated_mix__sliding_block_cached__dense_activation_gelu__decode_kernel(
    A_x, A_k_cache, A_v_cache, A_wq, A_wo, B_x, B_w1, B_b1, B_w2, B_b2, gate_w
):
    del B_x
    B, Sq, D = A_x.shape
    _, Hkv, Sk, Dh = A_k_cache.shape
    F = B_w1.shape[1]
    assert (B, Sq, Hkv, Dh) == (1, 1, _HQ, _DH)
    W = min(4096, max(256, Sk // 4))
    PW = 2 * Dh
    NPAIR = _HQ // 2
    HD = _HQ * Dh
    NCT = D // 128
    PC = 16 * 128
    M, NP = _M, _NP
    f32, bf16 = jnp.float32, jnp.bfloat16
    scale = Dh ** -0.5

    WQ_PPR = HD // PC
    WQ_NB = (D // 8) * WQ_PPR // 4
    WO_TILES = (HD // 8) * NCT
    WO_NB = WO_TILES // _TILE_BLK // 2
    WO_GB = WO_NB // _WO_GROUPS
    WO_GR = WO_GB * _TILE_BLK // NCT
    W2_OFF = [sum(_W2_CHUNKS[:c]) for c in range(len(_W2_CHUNKS))]
    W2_PIECE = 20
    W1_N = D // _W1_ROWS // 2
    assert HD % PC == 0 and (D // 8) * WQ_PPR == 4 * WQ_NB
    assert WO_TILES == 2 * _WO_GROUPS * WO_GB * _TILE_BLK and WO_GR * NCT == WO_GB * _TILE_BLK
    assert sum(_W2_CHUNKS) == (F // 8) * NCT and all(n % (2 * W2_PIECE) == 0 and n % (16 * NCT) == 0 for n in _W2_CHUNKS)
    assert D == 2 * W1_N * _W1_ROWS and W % 128 == 0 and 0 < _K_CUT[0] < W and 0 < _V_CUT[0] < W
    _check_perm(WQ_NB)
    _check_perm(WO_GB)

    def kernel(x_hbm, kt_hbm, vt_hbm, wq_hbm, wo_hbm, w1_hbm, b1_hbm, w2_hbm, b2_hbm, g_hbm,
               o_ref,
               xs, gs, b1s, b2s, w1s, wqs, kb, vb, wos, w2s, lhs,
               sem_small, sem_w1, sem_wq, sem_k, sem_v, sem_wo, sem_w2):

        def start_w1():
            def piece(i):
                for t in range(2):
                    r0 = pl.multiple_of((i + t * W1_N) * _W1_ROWS, 8)
                    pltpu.make_async_copy(w1_hbm.at[pl.ds(r0, _W1_ROWS), :], w1s.at[pl.ds(r0, _W1_ROWS), :],
                                          sem_w1.at[0]).start(priority=t)
            _loop(W1_N, piece)

        def start_wq():
            def block(i):
                for u in range(2):
                    for t in range(2):
                        k = lax.rem(2 * _perm(i, WQ_NB) + u + _BLK_PHASE, 2 * WQ_NB) + t * 2 * WQ_NB
                        r0 = pl.multiple_of((k // WQ_PPR) * 8, 8)
                        c0 = pl.multiple_of((k % WQ_PPR) * PC, 128)
                        pltpu.make_async_copy(wq_hbm.at[pl.ds(r0, 8), pl.ds(c0, PC)],
                                              wqs.at[pl.ds(r0, 8), pl.ds(c0, PC)],
                                              sem_wq.at[0]).start(priority=t)
            _loop(WQ_NB, block)

        def start_window(hbm, buf, sem, j, cut, t_lo):
            def rowgroup(i):
                r0 = pl.multiple_of(i * 8, 8)
                rs = pl.multiple_of(j * PW + i * 8, 8)
                for c0, c1, t in ((0, cut, t_lo), (cut, W, 1 - t_lo)):
                    pltpu.make_async_copy(hbm.at[pl.ds(rs, 8), pl.ds(Sk - W + c0, c1 - c0)],
                                          buf.at[pl.ds(r0, 8), pl.ds(c0, c1 - c0)], sem).start(priority=t)
            _loop(PW // 8, rowgroup)

        def start_pair(j, slot):
            start_window(kt_hbm, kb.at[slot], sem_k.at[slot], j, *_K_CUT)
            start_window(vt_hbm, vb.at[slot], sem_v.at[slot], j, *_V_CUT)

        def start_wo(g):
            def block(i):
                for u in range(2):
                    for t in range(2):
                        k = lax.rem(2 * _perm(i, WO_GB) + u + _BLK_PHASE, 2 * WO_GB)
                        t0 = pl.multiple_of(16 * k + _TILE_BLK * (g * WO_GB + t * WO_NB), 16)
                        pltpu.make_async_copy(wo_hbm.at[pl.ds(t0, 16)], wos.at[pl.ds(t0, 16)],
                                              sem_wo.at[2 * g + t]).start(priority=t)
            _loop(WO_GB, block)

        def start_w2():
            for c, (off, ntile) in enumerate(zip(W2_OFF, _W2_CHUNKS)):
                def piece(k, c=c, off=off, half=ntile // 2):
                    for t in range(2):
                        t0 = pl.multiple_of(off + t * half + k * W2_PIECE, 4)
                        pltpu.make_async_copy(w2_hbm.at[pl.ds(t0, W2_PIECE)], w2s.at[pl.ds(t0, W2_PIECE)],
                                              sem_w2.at[c]).start(priority=t)
                _loop(ntile // 2 // W2_PIECE, piece)

        def times_tile_rows(lhs_bf, buf, rg0, nrg):
            outs = []
            for ct in range(NCT):
                rhs = buf[pl.ds(rg0 * NCT + ct, nrg, stride=NCT)].reshape(nrg * 8, 128)
                outs.append(jnp.dot(lhs_bf, rhs, preferred_element_type=f32))
            return jnp.concatenate(outs, axis=1)

        small = [pltpu.make_async_copy(x_hbm, xs, sem_small.at[0]),
                 pltpu.make_async_copy(g_hbm, gs, sem_small.at[1]),
                 pltpu.make_async_copy(b1_hbm, b1s, sem_small.at[2]),
                 pltpu.make_async_copy(b2_hbm, b2s, sem_small.at[3])]
        for i, cp in enumerate(small):
            cp.start(priority=i % 2)
        start_wq()
        start_w1()
        start_pair(0, 0)

        for cp in small:
            cp.wait()
        xv = xs[0].astype(f32)
        g = jax.nn.sigmoid(jnp.sum(xv * gs[...].astype(f32).reshape(1, D), axis=-1, keepdims=True))
        x8 = jnp.broadcast_to(xv, (M, D)).astype(bf16)

        _wait_filled(w1s, sem_w1.at[0])
        h = jnp.dot(x8, w1s[...], preferred_element_type=f32) + b1s[...].astype(f32).reshape(1, F)
        h = jax.nn.gelu(h, approximate=True) * (1.0 - g)
        hb = jnp.where(lax.broadcasted_iota(jnp.int32, (M, F), 0) == 0, h, 0.0).astype(bf16)
        _wait_filled(wqs, sem_wq.at[0])

        for j in range(1, NP):
            start_pair(j, j)

        row = lax.broadcasted_iota(jnp.int32, (M, PW), 0)
        col = lax.broadcasted_iota(jnp.int32, (M, PW), 1)
        diag = ((row == 0) & (col < Dh)) | ((row == 1) & (col >= Dh))

        def pair(j, carry):
            slot = j % NP
            cols = pl.ds(pl.multiple_of(j * PW, 128), PW)
            _wait_filled(kb.at[slot], sem_k.at[slot])
            q = jnp.dot(x8, wqs[:, cols], preferred_element_type=f32)
            qd = jnp.where(diag, q, 0.0).astype(bf16)
            s = jnp.dot(qd, kb[slot], preferred_element_type=f32) * scale
            m = jnp.max(s, axis=-1, keepdims=True)
            p = jnp.exp(s - m)
            l = jnp.sum(p, axis=-1, keepdims=True)
            _wait_filled(vb.at[slot], sem_v.at[slot])
            o = lax.dot_general(p.astype(bf16), vb[slot], (((1,), (1,)), ((), ())),
                                preferred_element_type=f32)
            lhs[:, cols] = jnp.where(diag, o * (g / l), 0.0)

            @pl.when(j + NP < NPAIR)
            def _():
                start_pair(j + NP, slot)

            @pl.when(j + NP == NPAIR)
            def _():
                for grp in range(_WO_EARLY):
                    start_wo(grp)
            return carry

        lax.fori_loop(0, NPAIR, pair, 0)

        for grp in range(_WO_EARLY, _WO_GROUPS):
            start_wo(grp)
        start_w2()

        acc = jnp.zeros((M, D), f32)
        for grp in range(_WO_GROUPS):
            for t in range(2):
                blk0 = grp * WO_GB + t * WO_NB
                _wait_filled(wos.at[pl.ds(blk0 * _TILE_BLK, WO_GB * _TILE_BLK)], sem_wo.at[2 * grp + t])
            for t in range(2):
                rg0 = (grp * WO_GB + t * WO_NB) * _TILE_BLK // NCT
                acc = acc + times_tile_rows(lhs[:, rg0 * 8:(rg0 + WO_GR) * 8].astype(bf16), wos, rg0, WO_GR)
        for c, (off, ntile) in enumerate(zip(W2_OFF, _W2_CHUNKS)):
            _wait_filled(w2s.at[pl.ds(off, ntile)], sem_w2.at[c])
            rg0, nrg = off // NCT, ntile // NCT
            acc = acc + times_tile_rows(hb[:, rg0 * 8:(rg0 + nrg) * 8], w2s, rg0, nrg)

        res = jnp.sum(acc, axis=0, keepdims=True) + (1.0 - g) * b2s[...].astype(f32).reshape(1, D)
        o_ref[0] = res.astype(o_ref.dtype)

    kt = jnp.transpose(A_k_cache, (0, 1, 3, 2)).reshape(Hkv * Dh, Sk)
    vt = jnp.transpose(A_v_cache, (0, 1, 3, 2)).reshape(Hkv * Dh, Sk)
    wo_t, w2_t = _tile_view(A_wo), _tile_view(B_w2)
    hbm = pl.BlockSpec(memory_space=pl.ANY)
    DMA = pltpu.SemaphoreType.DMA
    return pl.pallas_call(
        kernel,
        out_shape=jax.ShapeDtypeStruct((1, 1, D), A_x.dtype),
        in_specs=[hbm] * 10,
        out_specs=pl.BlockSpec(memory_space=pltpu.VMEM),
        scratch_shapes=[
            pltpu.VMEM((1, 1, D), bf16), pltpu.VMEM((D,), bf16),
            pltpu.VMEM((F,), bf16), pltpu.VMEM((D,), bf16),
            pltpu.VMEM((D, F), bf16), pltpu.VMEM((D, HD), bf16),
            pltpu.VMEM((NP, PW, W), bf16), pltpu.VMEM((NP, PW, W), bf16),
            pltpu.VMEM(wo_t.shape, bf16), pltpu.VMEM(w2_t.shape, bf16),
            pltpu.VMEM((M, HD), f32),
            DMA((4,)), DMA((1,)), DMA((1,)), DMA((NP,)), DMA((NP,)),
            DMA((2 * _WO_GROUPS,)), DMA((len(_W2_CHUNKS),)),
        ],
        compiler_params=pltpu.CompilerParams(vmem_limit_bytes=64 << 20),
    )(A_x, kt, vt, A_wq, wo_t, B_w1, B_b1, w2_t, B_b2, gate_w)
```

```python
import jax
import jax.numpy as jnp
from jax import lax
from jax.experimental import pallas as pl
from jax.experimental.pallas import tpu as pltpu

_HQ, _DH = 32, 192
_M = 8
_NP = 2
_TILE_BLK = 32
_STRIDE = 8
_K_CUT = (2048, 0)
_V_CUT = (3072, 1)
_BLK_PHASE = 1
_WO_GROUPS = 3
_WO_EARLY = 2
_W2_CHUNKS = (640, 240, 80)
_W1_ROWS = 16


def _tile_view(w):
    R, C = w.shape
    return w.reshape(R // 8, 8, C // 128, 128).transpose(0, 2, 1, 3).reshape((R // 8) * (C // 128), 8, 128)


def _perm(i, n):
    return (_STRIDE * (i + 1)) % (n + 1) - 1


def _check_perm(n):
    assert sorted(_perm(i, n) for i in range(n)) == list(range(n)), n


def _loop(n, f):
    lax.fori_loop(0, n, lambda i, c: (f(i), c)[1], 0)


def _wait_filled(buf, sem):
    pltpu.make_async_copy(buf, buf, sem).wait()


@jax.jit
def pallas_gated_mix__sliding_block_cached__dense_activation_gelu__decode_kernel(
    A_x, A_k_cache, A_v_cache, A_wq, A_wo, B_x, B_w1, B_b1, B_w2, B_b2, gate_w
):
    del B_x
    B, Sq, D = A_x.shape
    _, Hkv, Sk, Dh = A_k_cache.shape
    F = B_w1.shape[1]
    assert (B, Sq, Hkv, Dh) == (1, 1, _HQ, _DH)
    W = min(4096, max(256, Sk // 4))
    PW = 2 * Dh
    NPAIR = _HQ // 2
    HD = _HQ * Dh
    NCT = D // 128
    PC = 16 * 128
    M, NP = _M, _NP
    f32, bf16 = jnp.float32, jnp.bfloat16
    scale = Dh ** -0.5

    WQ_PPR = HD // PC
    WQ_NB = (D // 8) * WQ_PPR // 4
    WO_TILES = (HD // 8) * NCT
    WO_NB = WO_TILES // _TILE_BLK // 2
    WO_GB = WO_NB // _WO_GROUPS
    WO_GR = WO_GB * _TILE_BLK // NCT
    W2_OFF = [sum(_W2_CHUNKS[:c]) for c in range(len(_W2_CHUNKS))]
    W2_PIECE = 20
    W1_N = D // _W1_ROWS // 2
    assert HD % PC == 0 and (D // 8) * WQ_PPR == 4 * WQ_NB
    assert WO_TILES == 2 * _WO_GROUPS * WO_GB * _TILE_BLK and WO_GR * NCT == WO_GB * _TILE_BLK
    assert sum(_W2_CHUNKS) == (F // 8) * NCT and all(n % (2 * W2_PIECE) == 0 and n % (16 * NCT) == 0 for n in _W2_CHUNKS)
    assert D == 2 * W1_N * _W1_ROWS and W % 128 == 0 and 0 < _K_CUT[0] < W and 0 < _V_CUT[0] < W
    _check_perm(WQ_NB)
    _check_perm(WO_GB)

    def kernel(x_hbm, kt_hbm, vt_hbm, wq_hbm, wo_hbm, w1_hbm, b1_hbm, w2_hbm, b2_hbm, g_hbm,
               o_ref,
               xs, gs, b1s, b2s, w1s, wqs, kb, vb, wos, w2s, lhs,
               sem_small, sem_w1, sem_wq, sem_k, sem_v, sem_wo, sem_w2):

        def start_w1():
            def piece(i):
                for t in range(2):
                    r0 = pl.multiple_of((i + t * W1_N) * _W1_ROWS, 8)
                    pltpu.make_async_copy(w1_hbm.at[pl.ds(r0, _W1_ROWS), :], w1s.at[pl.ds(r0, _W1_ROWS), :],
                                          sem_w1.at[0]).start(priority=t)
            _loop(W1_N, piece)

        def start_wq():
            def block(i):
                for u in range(2):
                    for t in range(2):
                        k = lax.rem(2 * _perm(i, WQ_NB) + u + _BLK_PHASE, 2 * WQ_NB) + t * 2 * WQ_NB
                        r0 = pl.multiple_of((k // WQ_PPR) * 8, 8)
                        c0 = pl.multiple_of((k % WQ_PPR) * PC, 128)
                        pltpu.make_async_copy(wq_hbm.at[pl.ds(r0, 8), pl.ds(c0, PC)],
                                              wqs.at[pl.ds(r0, 8), pl.ds(c0, PC)],
                                              sem_wq.at[0]).start(priority=t)
            _loop(WQ_NB, block)

        def start_window(hbm, buf, sem, j, cut, t_lo):
            def rowgroup(i):
                r0 = pl.multiple_of(i * 8, 8)
                rs = pl.multiple_of(j * PW + i * 8, 8)
                for c0, c1, t in ((0, cut, t_lo), (cut, W, 1 - t_lo)):
                    pltpu.make_async_copy(hbm.at[pl.ds(rs, 8), pl.ds(Sk - W + c0, c1 - c0)],
                                          buf.at[pl.ds(r0, 8), pl.ds(c0, c1 - c0)], sem).start(priority=t)
            _loop(PW // 8, rowgroup)

        def start_pair(j, slot):
            start_window(kt_hbm, kb.at[slot], sem_k.at[slot], j, *_K_CUT)
            start_window(vt_hbm, vb.at[slot], sem_v.at[slot], j, *_V_CUT)

        def start_wo(g):
            def block(i):
                for u in range(2):
                    for t in range(2):
                        k = lax.rem(2 * _perm(i, WO_GB) + u + _BLK_PHASE, 2 * WO_GB)
                        t0 = pl.multiple_of(16 * k + _TILE_BLK * (g * WO_GB + t * WO_NB), 16)
                        pltpu.make_async_copy(wo_hbm.at[pl.ds(t0, 16)], wos.at[pl.ds(t0, 16)],
                                              sem_wo.at[2 * g + t]).start(priority=t)
            _loop(WO_GB, block)

        def start_w2():
            for c, (off, ntile) in enumerate(zip(W2_OFF, _W2_CHUNKS)):
                def piece(k, c=c, off=off, half=ntile // 2):
                    for t in range(2):
                        t0 = pl.multiple_of(off + t * half + k * W2_PIECE, 4)
                        pltpu.make_async_copy(w2_hbm.at[pl.ds(t0, W2_PIECE)], w2s.at[pl.ds(t0, W2_PIECE)],
                                              sem_w2.at[c]).start(priority=t)
                _loop(ntile // 2 // W2_PIECE, piece)

        def times_tile_rows(lhs_bf, buf, rg0, nrg):
            tiles = buf[pl.ds(rg0 * NCT, nrg * NCT)].reshape(nrg, NCT, 8, 128)
            outs = [jnp.dot(lhs_bf, tiles[:, ct].reshape(nrg * 8, 128), preferred_element_type=f32)
                    for ct in range(NCT)]
            return jnp.concatenate(outs, axis=1)

        small = [pltpu.make_async_copy(x_hbm, xs, sem_small.at[0]),
                 pltpu.make_async_copy(g_hbm, gs, sem_small.at[1]),
                 pltpu.make_async_copy(b1_hbm, b1s, sem_small.at[2]),
                 pltpu.make_async_copy(b2_hbm, b2s, sem_small.at[3])]
        for i, cp in enumerate(small):
            cp.start(priority=i % 2)
        start_wq()
        start_w1()
        start_pair(0, 0)

        for cp in small:
            cp.wait()
        xv = xs[0].astype(f32)
        g = jax.nn.sigmoid(jnp.sum(xv * gs[...].astype(f32).reshape(1, D), axis=-1, keepdims=True))
        x8 = jnp.broadcast_to(xv, (M, D)).astype(bf16)

        _wait_filled(w1s, sem_w1.at[0])
        h = jnp.dot(x8, w1s[...], preferred_element_type=f32) + b1s[...].astype(f32).reshape(1, F)
        h = jax.nn.gelu(h, approximate=True) * (1.0 - g)
        hb = jnp.where(lax.broadcasted_iota(jnp.int32, (M, F), 0) == 0, h, 0.0).astype(bf16)
        _wait_filled(wqs, sem_wq.at[0])

        for j in range(1, NP):
            start_pair(j, j)

        row = lax.broadcasted_iota(jnp.int32, (M, PW), 0)
        col = lax.broadcasted_iota(jnp.int32, (M, PW), 1)
        diag = ((row == 0) & (col < Dh)) | ((row == 1) & (col >= Dh))

        def pair(j, carry):
            slot = j % NP
            cols = pl.ds(pl.multiple_of(j * PW, 128), PW)
            _wait_filled(kb.at[slot], sem_k.at[slot])
            q = jnp.dot(x8, wqs[:, cols], preferred_element_type=f32)
            qd = jnp.where(diag, q, 0.0).astype(bf16)
            s = jnp.dot(qd, kb[slot], preferred_element_type=f32) * scale
            m = jnp.max(s, axis=-1, keepdims=True)
            p = jnp.exp(s - m)
            l = jnp.sum(p, axis=-1, keepdims=True)
            _wait_filled(vb.at[slot], sem_v.at[slot])
            o = lax.dot_general(p.astype(bf16), vb[slot], (((1,), (1,)), ((), ())),
                                preferred_element_type=f32)
            lhs[:, cols] = jnp.where(diag, o * (g / l), 0.0)

            @pl.when(j + NP < NPAIR)
            def _():
                start_pair(j + NP, slot)

            @pl.when(j + NP == NPAIR)
            def _():
                for grp in range(_WO_EARLY):
                    start_wo(grp)
            return carry

        lax.fori_loop(0, NPAIR, pair, 0)

        for grp in range(_WO_EARLY, _WO_GROUPS):
            start_wo(grp)
        start_w2()

        acc = jnp.zeros((M, D), f32)
        for grp in range(_WO_GROUPS):
            for t in range(2):
                blk0 = grp * WO_GB + t * WO_NB
                _wait_filled(wos.at[pl.ds(blk0 * _TILE_BLK, WO_GB * _TILE_BLK)], sem_wo.at[2 * grp + t])
            for t in range(2):
                rg0 = (grp * WO_GB + t * WO_NB) * _TILE_BLK // NCT
                acc = acc + times_tile_rows(lhs[:, rg0 * 8:(rg0 + WO_GR) * 8].astype(bf16), wos, rg0, WO_GR)
        for c, (off, ntile) in enumerate(zip(W2_OFF, _W2_CHUNKS)):
            _wait_filled(w2s.at[pl.ds(off, ntile)], sem_w2.at[c])
            rg0, nrg = off // NCT, ntile // NCT
            acc = acc + times_tile_rows(hb[:, rg0 * 8:(rg0 + nrg) * 8], w2s, rg0, nrg)

        res = jnp.sum(acc, axis=0, keepdims=True) + (1.0 - g) * b2s[...].astype(f32).reshape(1, D)
        o_ref[0] = res.astype(o_ref.dtype)

    kt = jnp.transpose(A_k_cache, (0, 1, 3, 2)).reshape(Hkv * Dh, Sk)
    vt = jnp.transpose(A_v_cache, (0, 1, 3, 2)).reshape(Hkv * Dh, Sk)
    wo_t, w2_t = _tile_view(A_wo), _tile_view(B_w2)
    hbm = pl.BlockSpec(memory_space=pl.ANY)
    DMA = pltpu.SemaphoreType.DMA
    return pl.pallas_call(
        kernel,
        out_shape=jax.ShapeDtypeStruct((1, 1, D), A_x.dtype),
        in_specs=[hbm] * 10,
        out_specs=pl.BlockSpec(memory_space=pltpu.VMEM),
        scratch_shapes=[
            pltpu.VMEM((1, 1, D), bf16), pltpu.VMEM((D,), bf16),
            pltpu.VMEM((F,), bf16), pltpu.VMEM((D,), bf16),
            pltpu.VMEM((D, F), bf16), pltpu.VMEM((D, HD), bf16),
            pltpu.VMEM((NP, PW, W), bf16), pltpu.VMEM((NP, PW, W), bf16),
            pltpu.VMEM(wo_t.shape, bf16), pltpu.VMEM(w2_t.shape, bf16),
            pltpu.VMEM((M, HD), f32),
            DMA((4,)), DMA((1,)), DMA((1,)), DMA((NP,)), DMA((NP,)),
            DMA((2 * _WO_GROUPS,)), DMA((len(_W2_CHUNKS),)),
        ],
        compiler_params=pltpu.CompilerParams(vmem_limit_bytes=64 << 20),
    )(A_x, kt, vt, A_wq, wo_t, B_w1, B_b1, w2_t, B_b2, gate_w)
```
